```python
import jax
import jax.numpy as jnp

def _softmax(x, axis=-1):
    return jax.nn.softmax(x, axis=axis)
def _gelu(x):
    return jax.nn.gelu(x, approximate=True)
def _silu(x):
    return jax.nn.silu(x)
def _sigmoid(x):
    return jax.nn.sigmoid(x)
def _layernorm(x, axis=-1, eps=1e-5):
    m = jnp.mean(x, axis=axis, keepdims=True)
    v = jnp.var(x, axis=axis, keepdims=True)
    return (x - m) / jnp.sqrt(v + eps)
def _scatter_add(tgt, idx, src, axis=0):
    return tgt.at[idx].add(src)
def _segment_sum(src, seg, n):
    return jax.ops.segment_sum(src, seg, n)
class _Rng:
    def __init__(self, key):
        self._k = key
    def _next(self):
        self._k, sub = jax.random.split(self._k)
        return sub
    def normal(self, shape):
        return jax.random.normal(self._next(), shape, dtype=jnp.bfloat16)
    def randint(self, lo, hi, shape):
        return jax.random.randint(self._next(), shape, lo, hi, dtype=jnp.int32)
    def uniform(self, shape, lo=0.0, hi=1.0):
        return jax.random.uniform(self._next(), shape, jnp.bfloat16, lo, hi)
    def permutation(self, n):
        return jax.random.permutation(self._next(), n)


kernel_name = 'recurrent_scan__sliding_block_cached__moe_arch_mod__decode'

def setup_inputs():
    _rng = _Rng(jax.random.key(int.from_bytes(__import__("os").urandom(4), "little")))
    _w = (lambda a: (lambda t: t.astype(jnp.bfloat16) if jnp.issubdtype(t.dtype, jnp.floating) else t)(jnp.asarray(a)))
    def _A_setup():
        B, Sq, D = 1, 1, 512
        Hq, Hkv, Sk, Dh = 32, 32, 32768, 128
        assert Hq % Hkv == 0, (Hq, Hkv)
        return {
            "x": _w((lambda *s: _rng.normal(s) * 0.05)(B, Sq, D)),
            "k_cache": _w((lambda *s: _rng.normal(s) * 0.05)(B, Hkv, Sk, Dh)),
            "v_cache": _w((lambda *s: _rng.normal(s) * 0.05)(B, Hkv, Sk, Dh)),
            "wq": _w((lambda *s: _rng.normal(s) * 0.05)(D, Hq * Dh) * (D ** -0.5)),
            "wo": _w((lambda *s: _rng.normal(s) * 0.05)(Hq * Dh, D) * ((Hq * Dh) ** -0.5)),
        }
    _A_in = _A_setup()

    def _B_setup():
        B, S, D, F, C = 1, 1, 512, 1376, 1
        return {
            "x": _w((lambda *s: _rng.normal(s) * 0.05)(B, S, D)),
            "w_r": _w((lambda *s: _rng.normal(s) * 0.05)(D)),
            "w_gate": _w((lambda *s: _rng.normal(s) * 0.05)(D, F)),
            "w_up": _w((lambda *s: _rng.normal(s) * 0.05)(D, F)),
            "w_down": _w((lambda *s: _rng.normal(s) * 0.05)(F, D)),
        }
    _B_in = _B_setup()

    return {
        "A_x": _A_in["x"],
        "A_k_cache": _A_in["k_cache"],
        "A_v_cache": _A_in["v_cache"],
        "A_wq": _A_in["wq"],
        "A_wo": _A_in["wo"],
        "B_x": _B_in["x"],
        "B_w_r": _B_in["w_r"],
        "B_w_gate": _B_in["w_gate"],
        "B_w_up": _B_in["w_up"],
        "B_w_down": _B_in["w_down"],
    }

def reference(A_x, A_k_cache, A_v_cache, A_wq, A_wo, B_x, B_w_r, B_w_gate, B_w_up, B_w_down):
    def _A_ref(x, k_cache, v_cache, wq, wo):
        B, Sq, D = x.shape
        Hq, Dh = 32, 128
        Hkv, Sk = k_cache.shape[1], k_cache.shape[2]
        W = min(4096, max(256, Sk // 4))
        rep = Hq // Hkv
        q = (lambda x, *d: x.transpose(*d))((x @ wq).reshape(B, Sq, Hq, Dh), 0, 2, 1, 3)
        k = jnp.repeat(k_cache[:, :, Sk - W:, :], rep, axis=1)
        v = jnp.repeat(v_cache[:, :, Sk - W:, :], rep, axis=1)
        scores = jnp.einsum("bhqd,bhkd->bhqk", q, k) * (Dh ** -0.5)
        p = _softmax(scores, axis=-1)
        o = jnp.einsum("bhqk,bhkd->bhqd", p, v)
        return (lambda x, *d: x.transpose(*d))(o, 0, 2, 1, 3).reshape(B, Sq, Hq * Dh) @ wo

    def _B_ref(x, w_r, w_gate, w_up, w_down):
        B, S, D = x.shape
        C = 1
        r = x @ w_r
        idx = jnp.argsort(-r, axis=-1)[:, :C]
        idx_e = jnp.repeat(idx.reshape(B, C, 1), D, axis=2)
        x_sel = jnp.take_along_axis(x, idx_e, axis=1)
        g = _silu(x_sel @ w_gate)
        u = x_sel @ w_up
        y = (g * u) @ w_down
        r_sel = _sigmoid(jnp.take_along_axis(r, idx, axis=1))
        y = y * r_sel.reshape(B, C, 1)
        b_off = (jnp.arange(B) * S).reshape(B, 1)
        flat_idx = (idx + b_off).reshape(B * C)
        zero = (x * 0.0).reshape(B * S, D)
        upd = _scatter_add(zero, flat_idx, y.reshape(B * C, D), axis=0)
        return x + upd.reshape(B, S, D)

    x = A_x
    xn = _layernorm(x, axis=-1)
    s = _A_ref(xn, A_k_cache, A_v_cache, A_wq, A_wo)
    g = _silu(_B_ref(xn, B_w_r, B_w_gate, B_w_up, B_w_down))
    return x + s * g
```

```python
import functools
import jax
import jax.numpy as jnp
from jax import lax
import jax.experimental.pallas as pl
import jax.experimental.pallas.tpu as pltpu

D = 512
H = 32
DH = 128
F = 1376
SUB = 128
LOOK = 2
NT = (((1,), (1,)), ((), ()))
NN = (((1,), (0,)), ((), ()))
f32 = jnp.float32
bf16 = jnp.bfloat16


def _kernel(x_hbm, k_hbm, v_hbm, wq_hbm, wo_hbm, wr_hbm, wg_hbm, wu_hbm, wd_hbm,
            out_hbm,
            kb, vb, wqb, wob, wgb, wub, wdb, xb, wrb, qs, os_, ob, hsem, wsem,
            *, SK, W):
    base = SK - W

    def split2(src, dst, r0, nrows, rows_per, sem):
        half = nrows // 2
        n = -(-half // rows_per)
        for j in range(n):
            sz = min(rows_per, half - j * rows_per)
            for p in range(2):
                o = r0 + p * half + j * rows_per
                pltpu.make_async_copy(src.at[pl.ds(o, sz)], dst.at[pl.ds(o, sz)], sem).start(priority=p)

    def wait_rows(dst, r0, nrows, sem):
        d = dst.at[pl.ds(r0, nrows)]
        pltpu.make_async_copy(d, d, sem).wait()

    def start_head(h, slot):
        for j in range(W // SUB):
            pltpu.make_async_copy(k_hbm.at[0, h, pl.ds(base + j * SUB, SUB)], kb.at[h, pl.ds(j * SUB, SUB)], hsem.at[slot]).start(priority=0)
            pltpu.make_async_copy(v_hbm.at[0, h, pl.ds(base + j * SUB, SUB)], vb.at[h, pl.ds(j * SUB, SUB)], hsem.at[slot]).start(priority=1)

    def wait_head(h, slot):
        pltpu.make_async_copy(kb.at[h], kb.at[h], hsem.at[slot]).wait()
        pltpu.make_async_copy(vb.at[h], vb.at[h], hsem.at[slot]).wait()

    split2(wq_hbm, wqb, 0, D, 16, wsem.at[0])
    pltpu.make_async_copy(x_hbm, xb, wsem.at[0]).start()
    pltpu.make_async_copy(wr_hbm, wrb, wsem.at[0]).start()
    for j in range(F // 32):
        pltpu.make_async_copy(wg_hbm.at[pl.ds(j * 32, 32)], wgb.at[pl.ds(j * 32, 32)], wsem.at[1]).start(priority=0)
        pltpu.make_async_copy(wu_hbm.at[pl.ds(j * 32, 32)], wub.at[pl.ds(j * 32, 32)], wsem.at[1]).start(priority=1)
    start_head(0, 0)

    pltpu.make_async_copy(wqb, wqb, wsem.at[0]).wait()
    pltpu.make_async_copy(xb, xb, wsem.at[0]).wait()
    pltpu.make_async_copy(wrb, wrb, wsem.at[0]).wait()
    split2(wd_hbm, wdb, 0, F, 32, wsem.at[0])
    start_head(1, 1)

    x = xb[0].astype(f32)
    mean = jnp.mean(x, axis=-1, keepdims=True)
    xc = x - mean
    var = jnp.mean(xc * xc, axis=-1, keepdims=True)
    xn = (xc / jnp.sqrt(var + 1e-5)).astype(bf16)
    xnf = xn.astype(f32)
    qs[...] = lax.dot_general(xn, wqb[...], NN, preferred_element_type=f32)

    pltpu.make_async_copy(wgb, wgb, wsem.at[1]).wait()
    pltpu.make_async_copy(wub, wub, wsem.at[1]).wait()
    gate = lax.dot_general(xn, wgb[...], NT, preferred_element_type=f32)
    up = lax.dot_general(xn, wub[...], NT, preferred_element_type=f32)
    hmid = (gate * jax.nn.sigmoid(gate) * up).astype(bf16)
    pltpu.make_async_copy(wdb, wdb, wsem.at[0]).wait()
    y = lax.dot_general(hmid, wdb[...], NN, preferred_element_type=f32)
    wr = wrb[...].astype(f32).reshape(1, D)
    r = jnp.sum(xnf * wr, axis=-1, keepdims=True)
    y = y * jax.nn.sigmoid(r)
    z = xnf + (xnf * 0.0 + y)
    g = z * jax.nn.sigmoid(z)

    WO_CH = [(0, 2048), (2048, 1536), (3584, 384), (3968, 128)]

    def body(h, carry):
        slot = h % LOOK
        wait_head(h, slot)

        @pl.when(h + LOOK < H)
        def _():
            start_head(h + LOOK, slot)

        @pl.when(h + LOOK == H)
        def _():
            split2(wo_hbm, wob, WO_CH[0][0], WO_CH[0][1], 32, wsem.at[0])

        @pl.when(h + LOOK == H + 1)
        def _():
            split2(wo_hbm, wob, WO_CH[1][0], WO_CH[1][1], 32, wsem.at[1])
            split2(wo_hbm, wob, WO_CH[2][0], WO_CH[2][1], 32, wsem.at[2])
            split2(wo_hbm, wob, WO_CH[3][0], WO_CH[3][1], 32, wsem.at[3])

        off = pl.multiple_of(h * DH, DH)
        q = qs[:, pl.ds(off, DH)].astype(bf16)
        s = lax.dot_general(q, kb[h], NT, preferred_element_type=f32) * (DH ** -0.5)
        m = jnp.max(s, axis=-1, keepdims=True)
        p = jnp.exp(s - m)
        l = jnp.sum(p, axis=-1, keepdims=True)
        o = lax.dot_general(p.astype(bf16), vb[h], NN, preferred_element_type=f32)
        os_[:, pl.ds(off, DH)] = o / l
        return carry

    lax.fori_loop(0, H, body, 0)

    acc = jnp.zeros((1, D), f32)
    for i, (r0, n) in enumerate(WO_CH):
        wait_rows(wob, r0, n, wsem.at[i])
        acc = acc + lax.dot_general(os_[:, r0:r0 + n].astype(bf16), wob[r0:r0 + n, :], NN, preferred_element_type=f32)
    ob[...] = (x + acc * g).astype(bf16).reshape(1, 1, D)
    c = pltpu.make_async_copy(ob, out_hbm, hsem.at[0])
    c.start()
    c.wait()


@jax.jit
def pallas_recurrent_scan__sliding_block_cached__moe_arch_mod__decode_kernel(A_x, A_k_cache, A_v_cache, A_wq, A_wo, B_x, B_w_r, B_w_gate, B_w_up, B_w_down):
    SK = A_k_cache.shape[2]
    W = min(4096, max(256, SK // 4))
    hbm = pl.BlockSpec(memory_space=pltpu.HBM)
    return pl.pallas_call(
        functools.partial(_kernel, SK=SK, W=W),
        grid=(),
        in_specs=[hbm] * 9,
        out_specs=hbm,
        out_shape=jax.ShapeDtypeStruct((1, 1, D), bf16),
        scratch_shapes=[
            pltpu.VMEM((H, W, DH), bf16), pltpu.VMEM((H, W, DH), bf16),
            pltpu.VMEM((D, H * DH), bf16), pltpu.VMEM((H * DH, D), bf16),
            pltpu.VMEM((F, D), bf16), pltpu.VMEM((F, D), bf16), pltpu.VMEM((F, D), bf16),
            pltpu.VMEM((1, 1, D), bf16), pltpu.VMEM((D,), bf16),
            pltpu.VMEM((1, H * DH), f32), pltpu.VMEM((1, H * DH), f32),
            pltpu.VMEM((1, 1, D), bf16),
            pltpu.SemaphoreType.DMA((LOOK,)), pltpu.SemaphoreType.DMA((4,)),
        ],
        compiler_params=pltpu.CompilerParams(vmem_limit_bytes=100 * 1024 * 1024),
    )(A_x, A_k_cache, A_v_cache, A_wq, A_wo, B_w_r, B_w_gate.T, B_w_up.T, B_w_down)
```

```python
import functools
import jax
import jax.numpy as jnp
from jax import lax
import jax.experimental.pallas as pl
import jax.experimental.pallas.tpu as pltpu

D = 512
H = 32
DH = 128
F = 1376
NT = (((1,), (1,)), ((), ()))
NN = (((1,), (0,)), ((), ()))
f32 = jnp.float32
bf16 = jnp.bfloat16
NS = 3


def _kernel(x_hbm, k_hbm, v_hbm, wq_hbm, wo_hbm, wr_hbm, wg_hbm, wu_hbm, wd_hbm,
            out_hbm,
            kb, vb, wqb, wob, wgb, wub, wdb, xb, wrb, qs, os_, accs, ob, sem,
            *, SK, W, SUB, TAIL, COMPUTE, SCOPES, WQR):
    base = SK - W
    import contextlib
    scope = (lambda n: jax.named_scope(n)) if SCOPES else (lambda n: contextlib.nullcontext())
    NIN = H - sum(TAIL)

    def cp(src, dst, s, prio):
        pltpu.make_async_copy(src, dst, s).start(priority=prio)

    def wait(dst, s):
        pltpu.make_async_copy(dst, dst, s).wait()

    def halves(src, dst, r0, half, step, s):
        assert half % step == 0
        def b(j, c):
            o = pl.multiple_of(r0 + j * step, step)
            cp(src.at[pl.ds(o, step)], dst.at[pl.ds(o, step)], s, 0)
            o = pl.multiple_of(r0 + half + j * step, step)
            cp(src.at[pl.ds(o, step)], dst.at[pl.ds(o, step)], s, 1)
            return c
        lax.fori_loop(0, half // step, b, 0)

    def issue_wq(s):
        cp(x_hbm, xb, s, 0)
        cp(wr_hbm, wrb, s, 1)
        def b(j, c):
            for p in range(2):
                r = pl.multiple_of(p * (D // 2) + (j // 4) * 16, 16)
                c0 = pl.multiple_of((j % 4) * 1024, 1024)
                cp(wq_hbm.at[pl.ds(r, 16), pl.ds(c0, 1024)], wqb.at[pl.ds(r, 16), pl.ds(c0, 1024)], s, p)
            return c
        lax.fori_loop(0, 64, b, 0)

    def issue_gu(s):
        def b(j, c):
            o = pl.multiple_of(j * 32, 32)
            cp(wg_hbm.at[pl.ds(o, 32)], wgb.at[pl.ds(o, 32)], s, 0)
            cp(wu_hbm.at[pl.ds(o, 32)], wub.at[pl.ds(o, 32)], s, 1)
            return c
        lax.fori_loop(0, F // 32, b, 0)

    def issue_wd(s):
        halves(wd_hbm, wdb, 0, F // 2, 16 * 1 if False else 16, s) if False else None
        def b(j, c):
            for p in range(2):
                o = pl.multiple_of(p * (F // 2) + j * 32, 16)
                cp(wd_hbm.at[pl.ds(o, 32)], wdb.at[pl.ds(o, 32)], s, p)
            return c
        lax.fori_loop(0, 21, b, 0)
        for p in range(2):
            o = p * (F // 2) + 21 * 32
            cp(wd_hbm.at[pl.ds(o, 16)], wdb.at[pl.ds(o, 16)], s, p)

    def issue_head(h, s):
        def b(j, c):
            o = pl.multiple_of(j * SUB, SUB)
            cp(k_hbm.at[0, h, pl.ds(base + o, SUB)], kb.at[h, pl.ds(o, SUB)], s, 0)
            cp(v_hbm.at[0, h, pl.ds(base + o, SUB)], vb.at[h, pl.ds(o, SUB)], s, 1)
            return c
        lax.fori_loop(0, W // SUB, b, 0)

    def issue_wo(h0, nh, s):
        def b(j, c):
            r = pl.multiple_of((h0 + j) * DH, DH)
            for i in range(4):
                o = pl.multiple_of(r + i * 32, 32)
                cp(wo_hbm.at[pl.ds(o, 32)], wob.at[pl.ds(o, 32)], s, i // 2)
            return c
        if isinstance(nh, int) and nh == 1:
            b(0, 0)
        else:
            lax.fori_loop(0, nh, b, 0)

    issue_wq(sem.at[0])
    issue_gu(sem.at[1])
    issue_wd(sem.at[2])

    with scope("wait_wq"):
        wait(wqb, sem.at[0]); wait(xb, sem.at[0]); wait(wrb, sem.at[0])
    issue_head(0, sem.at[0])
    issue_wo(0, 1, sem.at[0])
    x = xb[0].astype(f32)
    rnd = lambda t: t.astype(bf16).astype(f32)
    mean = jnp.mean(x, axis=-1, keepdims=True)
    xc = x - mean
    var = jnp.mean(xc * xc, axis=-1, keepdims=True)
    xn = (xc / jnp.sqrt(var + 1e-5)).astype(bf16)
    xnf = xn.astype(f32)
    if 'q' in COMPUTE:
        qs[...] = lax.dot_general(xn, wqb[...], NN, preferred_element_type=f32)

    with scope("wait_gu"):
        wait(wgb, sem.at[1]); wait(wub, sem.at[1])
    issue_head(1, sem.at[1])
    issue_wo(1, 1, sem.at[1])
    gate = lax.dot_general(xn, wgb[...], NT, preferred_element_type=f32)
    up = lax.dot_general(xn, wub[...], NT, preferred_element_type=f32)
    hmid = (gate * jax.nn.sigmoid(gate) * up).astype(bf16)
    with scope("wait_wd"):
        wait(wdb, sem.at[2])
    issue_head(2, sem.at[2])
    issue_wo(2, 1, sem.at[2])
    y = lax.dot_general(hmid, wdb[...], NN, preferred_element_type=f32)
    wr = wrb[...].astype(f32).reshape(1, D)
    r = jnp.sum(xnf * wr, axis=-1, keepdims=True)
    y = y * jax.nn.sigmoid(r)
    z = xnf + (xnf * 0.0 + y)
    g = z * jax.nn.sigmoid(z)

    def oproj(h, o):
        r = pl.multiple_of(h * DH, DH)
        return lax.dot_general(o.astype(bf16), wob[pl.ds(r, DH), :], NN, preferred_element_type=f32)

    tail_start = [NIN + sum(TAIL[:i]) for i in range(len(TAIL))]

    def body(h, acc):
        slot = h % NS
        s_ = sem.at[slot]
        with scope("wait_head"):
            wait(kb.at[h], s_)
            wait(vb.at[h], s_)

            @pl.when(h < NIN)
            def _():
                wait(wob.at[pl.ds(0, DH)], s_)

        @pl.when(h + NS < H)
        def _():
            issue_head(h + NS, s_)

        @pl.when(h + NS < NIN)
        def _():
            issue_wo(h + NS, 1, s_)

        for i, nh in enumerate(TAIL):
            @pl.when(h + NS == H + i)
            def _():
                issue_wo(tail_start[i], nh, s_)

        if 'h' in COMPUTE:
            off = pl.multiple_of(h * DH, DH)
            q = qs[:, pl.ds(off, DH)].astype(bf16)
            s = lax.dot_general(q, kb[h], NT, preferred_element_type=f32) * (DH ** -0.5)
            m = jnp.max(s, axis=-1, keepdims=True)
            p = jnp.exp(s - m)
            l = jnp.sum(p, axis=-1, keepdims=True)
            o = lax.dot_general(p.astype(bf16), vb[h], NN, preferred_element_type=f32) / l
            os_[:, pl.ds(off, DH)] = o
            acc = lax.cond(h < NIN, lambda: acc + oproj(h, o), lambda: acc)
        return acc

    acc = lax.fori_loop(0, H, body, jnp.zeros((1, D), f32))

    for i, nh in enumerate(TAIL):
        slot = (H + i) % NS
        with scope("wait_wo"):
            wait(wob.at[pl.ds(0, nh * DH)], sem.at[slot])
        if 'h' in COMPUTE:
            lo, hi = tail_start[i] * DH, (tail_start[i] + nh) * DH
            acc = acc + lax.dot_general(os_[:, lo:hi].astype(bf16), wob[lo:hi, :], NN, preferred_element_type=f32)
    if 'h' not in COMPUTE:
        acc = acc + qs[:, 0:512]
    ob[...] = (x + acc * g).astype(bf16).reshape(1, 1, D)
    with scope("out"):
        c = pltpu.make_async_copy(ob, out_hbm, sem.at[0])
        c.start()
        c.wait()


def make(SUB=128, TAIL=(8, 2, 1), COMPUTE='qh', NOCHECK=False, SCOPES=False, WQR=16):
    @jax.jit
    def kernel(A_x, A_k_cache, A_v_cache, A_wq, A_wo, B_x, B_w_r, B_w_gate, B_w_up, B_w_down):
        SK = A_k_cache.shape[2]
        W = min(4096, max(256, SK // 4))
        hbm = pl.BlockSpec(memory_space=pltpu.HBM)
        return pl.pallas_call(
            functools.partial(_kernel, SK=SK, W=W, SUB=SUB, TAIL=TAIL, COMPUTE=COMPUTE, SCOPES=SCOPES, WQR=WQR),
            grid=(),
            in_specs=[hbm] * 9,
            out_specs=hbm,
            out_shape=jax.ShapeDtypeStruct((1, 1, D), bf16),
            scratch_shapes=[
                pltpu.VMEM((H, W, DH), bf16), pltpu.VMEM((H, W, DH), bf16),
                pltpu.VMEM((D, H * DH), bf16), pltpu.VMEM((H * DH, D), bf16),
                pltpu.VMEM((F, D), bf16), pltpu.VMEM((F, D), bf16), pltpu.VMEM((F, D), bf16),
                pltpu.VMEM((1, 1, D), bf16), pltpu.VMEM((D,), bf16),
                pltpu.VMEM((1, H * DH), f32), pltpu.VMEM((1, H * DH), f32), pltpu.VMEM((1, D), f32),
                pltpu.VMEM((1, 1, D), bf16),
                pltpu.SemaphoreType.DMA((NS,)),
            ],
            compiler_params=pltpu.CompilerParams(vmem_limit_bytes=100 * 1024 * 1024, disable_bounds_checks=NOCHECK),
        )(A_x, A_k_cache, A_v_cache, A_wq, A_wo, B_w_r, B_w_gate.T, B_w_up.T, B_w_down)
    return kernel

pallas_recurrent_scan__sliding_block_cached__moe_arch_mod__decode_kernel = make()
```

```python
import functools, contextlib
import jax
import jax.numpy as jnp
from jax import lax
import jax.experimental.pallas as pl
import jax.experimental.pallas.tpu as pltpu

D = 512
H = 32
DH = 128
F = 1376
HF = F // 2
NT = (((1,), (1,)), ((), ()))
NN = (((1,), (0,)), ((), ()))
f32 = jnp.float32
bf16 = jnp.bfloat16


def _kernel(x_hbm, k_hbm, v_hbm, wq_hbm, wo_hbm, wr_hbm, wg_hbm, wu_hbm, wd_hbm,
            out_hbm,
            kb, vb, wqb, wob, wgb, wub, wdb, xb, wrb, qs, os_, hs, gs, ob, sem,
            *, SK, W, G, GR, DG, LAGX, CHUNKS, SLOTS, COMPUTE, SCOPES, WQ, REGION):
    base = SK - W
    scope = (lambda n: jax.named_scope(n)) if SCOPES else (lambda n: contextlib.nullcontext())
    LAG = G + LAGX
    CH = W // G

    def cp(src, dst, s, prio):
        pltpu.make_async_copy(src, dst, s).start(priority=prio)

    def wait(dst, s):
        pltpu.make_async_copy(dst, dst, s).wait()

    def issue_wq(s):
        cp(x_hbm, xb, s, 0)
        cp(wr_hbm, wrb, s, 1)
        def b(j, c):
            r = pl.multiple_of((j // 16) * 16, 16)
            if WQ == 'a':
                for p in range(2):
                    c0 = pl.multiple_of(((j % 16) * 2 + p) * 128, 128)
                    cp(wq_hbm.at[:, pl.ds(r, 16), pl.ds(c0, 128)], wqb.at[:, pl.ds(r, 16), pl.ds(c0, 128)], s, p)
            else:
                c0 = pl.multiple_of(((j % 16) // 4) * 1024, 1024)
                sg = j % 4
                for p in range(2):
                    cp(wq_hbm.at[4 * p + sg, pl.ds(r, 16), pl.ds(c0, 1024)], wqb.at[4 * p + sg, pl.ds(r, 16), pl.ds(c0, 1024)], s, p)
            return c
        lax.fori_loop(0, 64, b, 0)

    def issue_gu(s):
        def b(j, c):
            r = pl.multiple_of(j * 16, 16)
            cp(wg_hbm.at[:, pl.ds(r, 16), :], wgb.at[:, pl.ds(r, 16), :], s, 0)
            cp(wu_hbm.at[:, pl.ds(r, 16), :], wub.at[:, pl.ds(r, 16), :], s, 1)
            return c
        lax.fori_loop(0, HF // 16, b, 0)

    def issue_wd(s):
        def b(j, c):
            for p in range(2):
                r = pl.multiple_of((2 * j + p) * 16, 16)
                cp(wd_hbm.at[:, pl.ds(r, 16), :], wdb.at[:, pl.ds(r, 16), :], s, p)
            return c
        lax.fori_loop(0, HF // 32, b, 0)
        r = HF // 32 * 32
        cp(wd_hbm.at[:, pl.ds(r, 16), :], wdb.at[:, pl.ds(r, 16), :], s, 0)

    def issue_kv(t, s):
        h0 = (t // G) * G
        r0 = (t % G) * CH
        def b(j, c):
            o = pl.multiple_of(r0 + j * GR, GR)
            for d in range(G // DG):
                hh = h0 + d * DG
                cp(k_hbm.at[0, pl.ds(hh, DG), pl.ds(base + o, GR), :], kb.at[pl.ds(hh, DG), pl.ds(o, GR), :], s, 0)
                cp(v_hbm.at[0, pl.ds(hh, DG), pl.ds(base + o, GR), :], vb.at[pl.ds(hh, DG), pl.ds(o, GR), :], s, 1)
            return c
        lax.fori_loop(0, CH // GR, b, 0)

    def issue_wo(h0, nh, s):
        def b(j, c):
            hh = h0 + j
            for i in range(4):
                cp(wo_hbm.at[hh, pl.ds(i * 32, 32), :], wob.at[hh, pl.ds(i * 32, 32), :], s, i % 2)
            return c
        lax.fori_loop(0, nh, b, 0)

    issue_wq(sem.at[0])
    issue_gu(sem.at[1])

    with scope("wait_wq"):
        wait(wqb, sem.at[0]); wait(xb, sem.at[0]); wait(wrb, sem.at[0])
    x = xb[0].astype(f32)
    mean = jnp.mean(x, axis=-1, keepdims=True)
    xc = x - mean
    var = jnp.mean(xc * xc, axis=-1, keepdims=True)
    xn = (xc / jnp.sqrt(var + 1e-5)).astype(bf16)
    qs[...] = lax.dot_general(xn, wqb[...].reshape(D, H * DH), NN, preferred_element_type=f32)

    def gate_up():
        with scope("wait_gu"):
            wait(wgb, sem.at[1]); wait(wub, sem.at[1])
        gate = lax.dot_general(xn, wgb[...].reshape(F, D), NT, preferred_element_type=f32)
        up = lax.dot_general(xn, wub[...].reshape(F, D), NT, preferred_element_type=f32)
        hs[...] = gate * jax.nn.sigmoid(gate) * up

    def down():
        with scope("wait_wd"):
            wait(wdb, sem.at[0])
        xnf = xn.astype(f32)
        y = lax.dot_general(hs[...].astype(bf16), wdb[...].reshape(F, D), NN, preferred_element_type=f32)
        wr = wrb[...].astype(f32).reshape(1, D)
        r = jnp.sum(xnf * wr, axis=-1, keepdims=True)
        y = y * jax.nn.sigmoid(r)
        z = xnf + (xnf * 0.0 + y)
        gs[...] = z * jax.nn.sigmoid(z)

    starts = [sum(CHUNKS[:i]) for i in range(len(CHUNKS))]
    def issue_slot(tt):
        for i, sl in enumerate(SLOTS):
            if sl == tt:
                issue_wo(starts[i], CHUNKS[i], sem.at[2 + i])

    def body(t, carry):
        @pl.when(t < H)
        def _():
            issue_kv(t, sem.at[(t // G) % 2])

        @pl.when(t == H)
        def _():
            issue_wd(sem.at[0])
            issue_slot(0)

        for tt in range(1, LAG):
            if tt in SLOTS:
                @pl.when(t == H + tt)
                def _():
                    issue_slot(tt)

        @pl.when(t == 1)
        def _():
            gate_up()

        h = t - LAG

        @pl.when(jnp.logical_and(h >= 0, h % G == 0))
        def _():
            with scope("wait_grp"):
                s_ = sem.at[(h // G) % 2]
                wait(kb.at[pl.ds(0, G)], s_)
                wait(vb.at[pl.ds(0, G)], s_)

        if 'h' in COMPUTE:
            @pl.when(h >= 0)
            def _():
                off = pl.multiple_of(h * DH, DH)
                q = qs[:, pl.ds(off, DH)].astype(bf16)
                s = lax.dot_general(q, kb[h], NT, preferred_element_type=f32) * (DH ** -0.5)
                m = jnp.max(s, axis=-1, keepdims=True)
                p = jnp.exp(s - m)
                l = jnp.sum(p, axis=-1, keepdims=True)
                o = lax.dot_general(p.astype(bf16), vb[h], NN, preferred_element_type=f32) / l
                os_[:, pl.ds(off, DH)] = o
        return carry + 1

    tcount = lax.fori_loop(0, H + LAG, body, 0)
    live = tcount > 0

    issue_slot(LAG)
    if REGION:
        pl.when(live)(down)
    else:
        down()
    issue_slot(LAG + 1)
    acc = jnp.zeros((1, D), f32)
    for i, nh in enumerate(CHUNKS):
        h0 = starts[i]
        with scope("wait_wo"):
            wait(wob.at[pl.ds(h0, nh)], sem.at[2 + i])
        if 'h' in COMPUTE:
            def step(a):
                return a + lax.dot_general(os_[:, h0 * DH:(h0 + nh) * DH].astype(bf16),
                                           wob[h0:h0 + nh].reshape(nh * DH, D), NN, preferred_element_type=f32)
            acc = lax.cond(live, step, lambda a: a, acc) if REGION else step(acc)
    if 'h' not in COMPUTE:
        acc = acc + qs[:, 0:512]
    ob[...] = (x + acc * gs[...]).astype(bf16).reshape(1, 1, D)
    with scope("out"):
        c = pltpu.make_async_copy(ob, out_hbm, sem.at[0])
        c.start()
        c.wait()


def make(G=4, GR=32, DG=4, LAGX=0, CHUNKS=(16, 4, 4, 4, 4), SLOTS=(0, 2, 3, 4, 5), COMPUTE='h', NOCHECK=False, SCOPES=False, WQ='c', REGION=True):
    assert sum(CHUNKS) == H and len(CHUNKS) == len(SLOTS)
    @jax.jit
    def kernel(A_x, A_k_cache, A_v_cache, A_wq, A_wo, B_x, B_w_r, B_w_gate, B_w_up, B_w_down):
        SK = A_k_cache.shape[2]
        W = min(4096, max(256, SK // 4))
        hbm = pl.BlockSpec(memory_space=pltpu.HBM)
        return pl.pallas_call(
            functools.partial(_kernel, SK=SK, W=W, G=G, GR=GR, DG=DG, LAGX=LAGX, CHUNKS=CHUNKS, SLOTS=SLOTS, COMPUTE=COMPUTE,
                              SCOPES=SCOPES, WQ=WQ, REGION=REGION),
            grid=(),
            in_specs=[hbm] * 9,
            out_specs=hbm,
            out_shape=jax.ShapeDtypeStruct((1, 1, D), bf16),
            scratch_shapes=[
                pltpu.VMEM((H, W, DH), bf16), pltpu.VMEM((H, W, DH), bf16),
                pltpu.VMEM((8, 64, H * DH), bf16), pltpu.VMEM((H, DH, D), bf16),
                pltpu.VMEM((2, HF, D), bf16), pltpu.VMEM((2, HF, D), bf16), pltpu.VMEM((2, HF, D), bf16),
                pltpu.VMEM((1, 1, D), bf16), pltpu.VMEM((D,), bf16),
                pltpu.VMEM((1, H * DH), f32), pltpu.VMEM((1, H * DH), f32), pltpu.VMEM((1, F), f32), pltpu.VMEM((1, D), f32),
                pltpu.VMEM((1, 1, D), bf16),
                pltpu.SemaphoreType.DMA((2 + len(CHUNKS),)),
            ],
            compiler_params=pltpu.CompilerParams(vmem_limit_bytes=100 * 1024 * 1024, disable_bounds_checks=NOCHECK),
        )(A_x, A_k_cache, A_v_cache, A_wq.reshape(8, 64, H * DH), A_wo.reshape(H, DH, D), B_w_r,
          B_w_gate.T.reshape(2, HF, D), B_w_up.T.reshape(2, HF, D), B_w_down.reshape(2, HF, D))
    return kernel

pallas_recurrent_scan__sliding_block_cached__moe_arch_mod__decode_kernel = make()
```

```python
import functools, contextlib
import jax
import jax.numpy as jnp
from jax import lax
import jax.experimental.pallas as pl
import jax.experimental.pallas.tpu as pltpu

D = 512
H = 32
DH = 128
F = 1376
HF = F // 2
NT = (((1,), (1,)), ((), ()))
NN = (((1,), (0,)), ((), ()))
f32 = jnp.float32
bf16 = jnp.bfloat16


def _kernel(x_hbm, k_hbm, v_hbm, wq_hbm, wo_hbm, wr_hbm, wg_hbm, wu_hbm, wd_hbm,
            out_hbm,
            kb, vb, wqb, wob, wgb, wub, wdb, xb, wrb, qs, os_, hs, gs, ob, sem,
            *, SK, W, G, GR, DG, LAGX, CHUNKS, SLOTS, GU_SLOT, WD_SLOT, COMPUTE, SCOPES, WQ, PRE, VREV):
    base = SK - W
    scope = (lambda n: jax.named_scope(n)) if SCOPES else (lambda n: contextlib.nullcontext())
    LAG = 5
    CH = W // G
    NGRP = 5
    gu_tail = GU_SLOT is not None
    S_WQ = 2
    S_GU = (NGRP % 2) if gu_tail else 3
    S_WD = ((NGRP - 1) % 2) if gu_tail else (NGRP % 2)
    if gu_tail:
        assert WD_SLOT > LAGX
    S_WO = [2 + i for i in range(len(CHUNKS))]

    def cp(src, dst, s, prio):
        pltpu.make_async_copy(src, dst, s).start(priority=prio)

    def wait(dst, s):
        pltpu.make_async_copy(dst, dst, s).wait()

    def issue_wq(s):
        cp(x_hbm, xb, s, 0)
        cp(wr_hbm, wrb, s, 1)
        def b(j, c):
            r = pl.multiple_of((j // 16) * 16, 16)
            if WQ == 'c':
                c0 = pl.multiple_of(((j % 16) // 4) * 1024, 1024)
                sg = j % 4
                for p in range(2):
                    cp(wq_hbm.at[4 * p + sg, pl.ds(r, 16), pl.ds(c0, 1024)], wqb.at[4 * p + sg, pl.ds(r, 16), pl.ds(c0, 1024)], s, p)
            elif WQ == 'd':
                c0 = pl.multiple_of(((j % 16) // 2) * 512, 512)
                sg = j % 2
                for p in range(2):
                    cp(wq_hbm.at[pl.ds(4 * p + 2 * sg, 2), pl.ds(r, 16), pl.ds(c0, 512)], wqb.at[pl.ds(4 * p + 2 * sg, 2), pl.ds(r, 16), pl.ds(c0, 512)], s, p)
            return c
        lax.fori_loop(0, 64, b, 0)

    def issue_gu(s):
        def b(j, c):
            r = pl.multiple_of(j * 16, 16)
            cp(wg_hbm.at[:, pl.ds(r, 16), :], wgb.at[:, pl.ds(r, 16), :], s, 0)
            cp(wu_hbm.at[:, pl.ds(r, 16), :], wub.at[:, pl.ds(r, 16), :], s, 1)
            return c
        lax.fori_loop(0, HF // 16, b, 0)

    def issue_wd(s):
        def b(j, c):
            for p in range(2):
                r = pl.multiple_of((2 * j + p) * 16, 16)
                cp(wd_hbm.at[:, pl.ds(r, 16), :], wdb.at[:, pl.ds(r, 16), :], s, p)
            return c
        lax.fori_loop(0, HF // 32, b, 0)
        r = HF // 32 * 32
        cp(wd_hbm.at[:, pl.ds(r, 16), :], wdb.at[:, pl.ds(r, 16), :], s, 0)

    def issue_kv_slice(h0, r0, ng, s):
        def b(j, c):
            o = pl.multiple_of(r0 + j * GR, GR)
            for d in range(ng // DG):
                hh = h0 + d * DG
                cp(k_hbm.at[0, pl.ds(hh, DG), pl.ds(base + o, GR), :], kb.at[pl.ds(hh, DG), pl.ds(o, GR), :], s, 0)
                cp(v_hbm.at[0, pl.ds(hh, DG), pl.ds(base + o, GR), :], vb.at[pl.ds(hh, DG), pl.ds(o, GR), :], s, 1)
            return c
        lax.fori_loop(0, W // ng // GR, b, 0)

    N8 = 24
    def kv_sem(hh):
        return sem.at[jnp.where(hh < N8, hh // 8, N8 // 8 + (hh - N8) // 4) % 2]

    def issue_kv8(t):
        issue_kv_slice((t // 8) * 8, (t % 8) * (W // 8), 8, kv_sem(t))

    def issue_kv4(t):
        issue_kv_slice((t // 4) * 4, (t % 4) * (W // 4), 4, kv_sem(t))

    def issue_wo(h0, nh, s):
        def b(j, c):
            hh = h0 + j
            for i in range(4):
                cp(wo_hbm.at[hh, pl.ds(i * 32, 32), :], wob.at[hh, pl.ds(i * 32, 32), :], s, i % 2)
            return c
        lax.fori_loop(0, nh, b, 0)

    issue_wq(sem.at[S_WQ])
    if not gu_tail:
        issue_gu(sem.at[S_GU])
    for t0 in range(PRE):
        issue_kv_slice(0, t0 * (W // 8), 8, sem.at[0])

    with scope("wait_wq"):
        wait(wqb, sem.at[S_WQ]); wait(xb, sem.at[S_WQ]); wait(wrb, sem.at[S_WQ])
    x = xb[0].astype(f32)
    mean = jnp.mean(x, axis=-1, keepdims=True)
    xc = x - mean
    var = jnp.mean(xc * xc, axis=-1, keepdims=True)
    xn = (xc / jnp.sqrt(var + 1e-5)).astype(bf16)
    s_scale = DH ** -0.5
    qs[...] = lax.dot_general(xn, wqb[...].reshape(D, H * DH), NN, preferred_element_type=f32)

    def gate_up():
        with scope("wait_gu"):
            wait(wgb, sem.at[S_GU]); wait(wub, sem.at[S_GU])
        gate = lax.dot_general(xn, wgb[...].reshape(F, D), NT, preferred_element_type=f32)
        up = lax.dot_general(xn, wub[...].reshape(F, D), NT, preferred_element_type=f32)
        hs[...] = gate * jax.nn.sigmoid(gate) * up

    def down():
        with scope("wait_wd"):
            wait(wdb, sem.at[S_WD])
        xnf = xn.astype(f32)
        y = lax.dot_general(hs[...].astype(bf16), wdb[...].reshape(F, D), NN, preferred_element_type=f32)
        wr = wrb[...].astype(f32).reshape(1, D)
        r = jnp.sum(xnf * wr, axis=-1, keepdims=True)
        y = y * jax.nn.sigmoid(r)
        z = xnf + (xnf * 0.0 + y)
        gs[...] = z * jax.nn.sigmoid(z)

    starts = [sum(CHUNKS[:i]) for i in range(len(CHUNKS))]

    def issue_slot(tt):
        if gu_tail and GU_SLOT == tt:
            issue_gu(sem.at[S_GU])
        if WD_SLOT == tt:
            issue_wd(sem.at[S_WD])
        for i, sl in enumerate(SLOTS):
            if sl == tt:
                issue_wo(starts[i], CHUNKS[i], sem.at[S_WO[i]])

    used_slots = set(SLOTS) | {WD_SLOT} | ({GU_SLOT} if gu_tail else set())

    def body(t, carry):
        @pl.when(jnp.logical_and(t >= PRE, t < N8))
        def _():
            issue_kv8(t)

        @pl.when(jnp.logical_and(t >= N8, t < H))
        def _():
            issue_kv4(t)

        for tt in range(LAG):
            if tt in used_slots:
                @pl.when(t == H + tt)
                def _():
                    issue_slot(tt)

        if not gu_tail:
            @pl.when(t == 1)
            def _():
                gate_up()

        def done(u):
            return jnp.where(u <= 25, jnp.maximum(u - 9, 0), jnp.where(u <= 29, 16 + 2 * (u - 25), 24 + (u - 29)))

        def head(h, c):
            @pl.when(jnp.logical_or(jnp.logical_and(h < N8, h % 8 == 0), jnp.logical_and(h >= N8, h % 4 == 0)))
            def _():
                with scope("wait_grp"):
                    s_ = kv_sem(h)
                    wait(kb.at[pl.ds(0, 4)], s_)
                    wait(vb.at[pl.ds(0, 4)], s_)

                    @pl.when(h < N8)
                    def _():
                        wait(kb.at[pl.ds(0, 4)], s_)
                        wait(vb.at[pl.ds(0, 4)], s_)

            if 'h' in COMPUTE:
                off = pl.multiple_of(h * DH, DH)
                q = qs[:, pl.ds(off, DH)].astype(bf16)
                s = lax.dot_general(q, kb[h], NT, preferred_element_type=f32) * s_scale
                m = jnp.max(s, axis=-1, keepdims=True)
                p = jnp.exp(s - m)
                l = jnp.sum(p, axis=-1, keepdims=True)
                o = lax.dot_general(p.astype(bf16), vb[h], NN, preferred_element_type=f32) / l
                os_[:, pl.ds(off, DH)] = o
            return c

        lax.fori_loop(done(t), done(t + 1), head, 0)
        return carry + 1

    tcount = lax.fori_loop(0, 37, body, 0)
    live = tcount > 0

    issue_slot(LAG)
    if gu_tail:
        pl.when(live)(gate_up)
        issue_slot(LAG + 1)
    pl.when(live)(down)
    issue_slot(LAG + 1 + (1 if gu_tail else 0))
    acc = jnp.zeros((1, D), f32)
    for i, nh in enumerate(CHUNKS):
        h0 = starts[i]
        with scope("wait_wo"):
            wait(wob.at[pl.ds(h0, nh)], sem.at[S_WO[i]])
        if 'h' in COMPUTE:
            def step(a):
                return a + lax.dot_general(os_[:, h0 * DH:(h0 + nh) * DH].astype(bf16),
                                           wob[h0:h0 + nh].reshape(nh * DH, D), NN, preferred_element_type=f32)
            acc = lax.cond(live, step, lambda a: a, acc)
    if 'h' not in COMPUTE:
        acc = acc + qs[:, 0:512]
    ob[...] = (x + acc * gs[...]).astype(bf16).reshape(1, 1, D)
    with scope("out"):
        c = pltpu.make_async_copy(ob, out_hbm, sem.at[0])
        c.start()
        c.wait()


def make(G=4, GR=64, DG=2, LAGX=1, CHUNKS=(16, 8, 4, 2, 2), SLOTS=(0, 2, 4, 5, 5), GU_SLOT=None, WD_SLOT=0,
         COMPUTE='h', NOCHECK=False, SCOPES=False, WQ='c', PRE=1, VREV=0):
    assert sum(CHUNKS) == H and len(CHUNKS) == len(SLOTS)
    nsem = max(4, 2 + len(CHUNKS))
    @jax.jit
    def kernel(A_x, A_k_cache, A_v_cache, A_wq, A_wo, B_x, B_w_r, B_w_gate, B_w_up, B_w_down):
        SK = A_k_cache.shape[2]
        W = min(4096, max(256, SK // 4))
        hbm = pl.BlockSpec(memory_space=pltpu.HBM)
        return pl.pallas_call(
            functools.partial(_kernel, SK=SK, W=W, G=G, GR=GR, DG=DG, LAGX=LAGX, CHUNKS=CHUNKS, SLOTS=SLOTS,
                              GU_SLOT=GU_SLOT, WD_SLOT=WD_SLOT, COMPUTE=COMPUTE, SCOPES=SCOPES, WQ=WQ, PRE=PRE, VREV=VREV),
            grid=(),
            in_specs=[hbm] * 9,
            out_specs=hbm,
            out_shape=jax.ShapeDtypeStruct((1, 1, D), bf16),
            scratch_shapes=[
                pltpu.VMEM((H, W, DH), bf16), pltpu.VMEM((H, W, DH), bf16),
                pltpu.VMEM((8, 64, H * DH), bf16), pltpu.VMEM((H, DH, D), bf16),
                pltpu.VMEM((2, HF, D), bf16), pltpu.VMEM((2, HF, D), bf16), pltpu.VMEM((2, HF, D), bf16),
                pltpu.VMEM((1, 1, D), bf16), pltpu.VMEM((D,), bf16),
                pltpu.VMEM((1, H * DH), f32), pltpu.VMEM((1, H * DH), f32), pltpu.VMEM((1, F), f32), pltpu.VMEM((1, D), f32),
                pltpu.VMEM((1, 1, D), bf16),
                pltpu.SemaphoreType.DMA((nsem,)),
            ],
            compiler_params=pltpu.CompilerParams(vmem_limit_bytes=100 * 1024 * 1024, disable_bounds_checks=NOCHECK),
        )(A_x, A_k_cache, A_v_cache, A_wq.reshape(8, 64, H * DH), A_wo.reshape(H, DH, D), B_w_r,
          B_w_gate.T.reshape(2, HF, D), B_w_up.T.reshape(2, HF, D), B_w_down.reshape(2, HF, D))
    return kernel

pallas_recurrent_scan__sliding_block_cached__moe_arch_mod__decode_kernel = make()
```

```python
import functools, contextlib
import jax
import jax.numpy as jnp
from jax import lax
import jax.experimental.pallas as pl
import jax.experimental.pallas.tpu as pltpu

D = 512
H = 32
DH = 128
F = 1376
HF = F // 2
NT = (((1,), (1,)), ((), ()))
NN = (((1,), (0,)), ((), ()))
f32 = jnp.float32
bf16 = jnp.bfloat16


def _kernel(x_hbm, k_hbm, v_hbm, wq_hbm, wo_hbm, wr_hbm, wg_hbm, wu_hbm, wd_hbm,
            out_hbm,
            kb, vb, wqb, wob, wgb, wub, wdb, xb, wrb, qs, os_, hs, gs, ob, sem,
            *, SK, W, G, GR, DG, LAGX, CHUNKS, SLOTS, GU_SLOT, WD_SLOT, COMPUTE, SCOPES, WQ, PRE, VREV, WOPAT):
    base = SK - W
    scope = (lambda n: jax.named_scope(n)) if SCOPES else (lambda n: contextlib.nullcontext())
    LAG = 5
    CH = W // G
    NGRP = 5
    gu_tail = GU_SLOT is not None
    S_WQ = 2
    S_GU = (NGRP % 2) if gu_tail else 3
    S_WD = ((NGRP - 1) % 2) if gu_tail else (NGRP % 2)
    if gu_tail:
        assert WD_SLOT > LAGX
    S_WO = [2 + i for i in range(len(CHUNKS))]

    def cp(src, dst, s, prio):
        pltpu.make_async_copy(src, dst, s).start(priority=prio)

    def wait(dst, s):
        pltpu.make_async_copy(dst, dst, s).wait()

    def issue_wq(s):
        cp(x_hbm, xb, s, 0)
        cp(wr_hbm, wrb, s, 1)
        def b(j, c):
            r = pl.multiple_of((j // 16) * 16, 16)
            if WQ == 'c':
                c0 = pl.multiple_of(((j % 16) // 4) * 1024, 1024)
                sg = j % 4
                for p in range(2):
                    cp(wq_hbm.at[4 * p + sg, pl.ds(r, 16), pl.ds(c0, 1024)], wqb.at[4 * p + sg, pl.ds(r, 16), pl.ds(c0, 1024)], s, p)
            elif WQ == 'd':
                c0 = pl.multiple_of(((j % 16) // 2) * 512, 512)
                sg = j % 2
                for p in range(2):
                    cp(wq_hbm.at[pl.ds(4 * p + 2 * sg, 2), pl.ds(r, 16), pl.ds(c0, 512)], wqb.at[pl.ds(4 * p + 2 * sg, 2), pl.ds(r, 16), pl.ds(c0, 512)], s, p)
            return c
        lax.fori_loop(0, 64, b, 0)

    def issue_gu(s):
        def b(j, c):
            r = pl.multiple_of(j * 16, 16)
            cp(wg_hbm.at[:, pl.ds(r, 16), :], wgb.at[:, pl.ds(r, 16), :], s, 0)
            cp(wu_hbm.at[:, pl.ds(r, 16), :], wub.at[:, pl.ds(r, 16), :], s, 1)
            return c
        lax.fori_loop(0, HF // 16, b, 0)

    def issue_wd(s):
        def b(j, c):
            for p in range(2):
                r = pl.multiple_of((2 * j + p) * 16, 16)
                cp(wd_hbm.at[:, pl.ds(r, 16), :], wdb.at[:, pl.ds(r, 16), :], s, p)
            return c
        lax.fori_loop(0, HF // 32, b, 0)
        r = HF // 32 * 32
        cp(wd_hbm.at[:, pl.ds(r, 16), :], wdb.at[:, pl.ds(r, 16), :], s, 0)

    def issue_kv_slice(h0, r0, ng, s):
        def b(j, c):
            o = pl.multiple_of(r0 + j * GR, GR)
            for d in range(ng // DG):
                hh = h0 + d * DG
                cp(k_hbm.at[0, pl.ds(hh, DG), pl.ds(base + o, GR), :], kb.at[pl.ds(hh, DG), pl.ds(o, GR), :], s, 0)
                cp(v_hbm.at[0, pl.ds(hh, DG), pl.ds(base + o, GR), :], vb.at[pl.ds(hh, DG), pl.ds(o, GR), :], s, 1)
            return c
        lax.fori_loop(0, W // ng // GR, b, 0)

    N8 = 24
    def kv_sem(hh):
        return sem.at[jnp.where(hh < N8, hh // 8, N8 // 8 + (hh - N8) // 4) % 2]

    def issue_kv8(t):
        issue_kv_slice((t // 8) * 8, (t % 8) * (W // 8), 8, kv_sem(t))

    def issue_kv4(t):
        issue_kv_slice((t // 4) * 4, (t % 4) * (W // 4), 4, kv_sem(t))

    def issue_wo(h0, nh, s):
        sg0 = h0 // 4
        if WOPAT == 'seg' and nh == 16:
            def b(j, c):
                r = pl.multiple_of(j * 16, 16)
                for p in range(2):
                    cp(wo_hbm.at[pl.ds(sg0 + 2 * p, 2), pl.ds(r, 16), :], wob.at[pl.ds(sg0 + 2 * p, 2), pl.ds(r, 16), :], s, p)
                return c
            lax.fori_loop(0, 32, b, 0)
        elif WOPAT == 'seg' and nh == 8:
            def b(j, c):
                for p in range(2):
                    r = pl.multiple_of((2 * j + p) * 16, 16)
                    cp(wo_hbm.at[pl.ds(sg0, 2), pl.ds(r, 16), :], wob.at[pl.ds(sg0, 2), pl.ds(r, 16), :], s, p)
                return c
            lax.fori_loop(0, 16, b, 0)
        else:
            assert (h0 * DH) % 32 == 0
            def b(j, c):
                for p in range(2):
                    row = h0 * DH + (2 * j + p) * 32
                    sg = row // 512
                    r = pl.multiple_of(row % 512, 32)
                    cp(wo_hbm.at[sg, pl.ds(r, 32), :], wob.at[sg, pl.ds(r, 32), :], s, p)
                return c
            lax.fori_loop(0, nh * 2, b, 0)

    def wo_rows(h0, nh):
        sg0, r0 = (h0 * DH) // 512, (h0 * DH) % 512
        if nh % 4 == 0:
            return wob[sg0:sg0 + nh // 4].reshape(nh * DH, D)
        return wob[sg0, r0:r0 + nh * DH, :]

    def wo_wait_view(h0, nh):
        sg0, r0 = (h0 * DH) // 512, (h0 * DH) % 512
        if nh % 4 == 0:
            return wob.at[pl.ds(sg0, nh // 4)]
        return wob.at[sg0, pl.ds(r0, nh * DH), :]

    issue_wq(sem.at[S_WQ])
    if not gu_tail:
        issue_gu(sem.at[S_GU])
    for t0 in range(PRE):
        issue_kv_slice(0, t0 * (W // 8), 8, sem.at[0])

    with scope("wait_wq"):
        wait(wqb, sem.at[S_WQ]); wait(xb, sem.at[S_WQ]); wait(wrb, sem.at[S_WQ])
    x = xb[0].astype(f32)
    mean = jnp.mean(x, axis=-1, keepdims=True)
    xc = x - mean
    var = jnp.mean(xc * xc, axis=-1, keepdims=True)
    xn = (xc / jnp.sqrt(var + 1e-5)).astype(bf16)
    s_scale = DH ** -0.5
    qs[...] = lax.dot_general(xn, wqb[...].reshape(D, H * DH), NN, preferred_element_type=f32)

    def gate_up():
        with scope("wait_gu"):
            wait(wgb, sem.at[S_GU]); wait(wub, sem.at[S_GU])
        gate = lax.dot_general(xn, wgb[...].reshape(F, D), NT, preferred_element_type=f32)
        up = lax.dot_general(xn, wub[...].reshape(F, D), NT, preferred_element_type=f32)
        hs[...] = gate * jax.nn.sigmoid(gate) * up

    def down():
        with scope("wait_wd"):
            wait(wdb, sem.at[S_WD])
        xnf = xn.astype(f32)
        y = lax.dot_general(hs[...].astype(bf16), wdb[...].reshape(F, D), NN, preferred_element_type=f32)
        wr = wrb[...].astype(f32).reshape(1, D)
        r = jnp.sum(xnf * wr, axis=-1, keepdims=True)
        y = y * jax.nn.sigmoid(r)
        z = xnf + (xnf * 0.0 + y)
        gs[...] = z * jax.nn.sigmoid(z)

    starts = [sum(CHUNKS[:i]) for i in range(len(CHUNKS))]

    def issue_slot(tt):
        if gu_tail and GU_SLOT == tt:
            issue_gu(sem.at[S_GU])
        if WD_SLOT == tt:
            issue_wd(sem.at[S_WD])
        for i, sl in enumerate(SLOTS):
            if sl == tt:
                issue_wo(starts[i], CHUNKS[i], sem.at[S_WO[i]])

    used_slots = set(SLOTS) | {WD_SLOT} | ({GU_SLOT} if gu_tail else set())

    def body(t, carry):
        @pl.when(jnp.logical_and(t >= PRE, t < N8))
        def _():
            issue_kv8(t)

        @pl.when(jnp.logical_and(t >= N8, t < H))
        def _():
            issue_kv4(t)

        for tt in range(LAG):
            if tt in used_slots:
                @pl.when(t == H + tt)
                def _():
                    issue_slot(tt)

        if not gu_tail:
            @pl.when(t == 1)
            def _():
                gate_up()

        def done(u):
            return jnp.where(u <= 25, jnp.maximum(u - 9, 0), jnp.where(u <= 29, 16 + 2 * (u - 25), 24 + (u - 29)))

        def head(h, c):
            @pl.when(jnp.logical_or(jnp.logical_and(h < N8, h % 8 == 0), jnp.logical_and(h >= N8, h % 4 == 0)))
            def _():
                with scope("wait_grp"):
                    s_ = kv_sem(h)
                    wait(kb.at[pl.ds(0, 4)], s_)
                    wait(vb.at[pl.ds(0, 4)], s_)

                    @pl.when(h < N8)
                    def _():
                        wait(kb.at[pl.ds(0, 4)], s_)
                        wait(vb.at[pl.ds(0, 4)], s_)

            if 'h' in COMPUTE:
                off = pl.multiple_of(h * DH, DH)
                q = qs[:, pl.ds(off, DH)].astype(bf16)
                s = lax.dot_general(q, kb[h], NT, preferred_element_type=f32) * s_scale
                m = jnp.max(s, axis=-1, keepdims=True)
                p = jnp.exp(s - m)
                l = jnp.sum(p, axis=-1, keepdims=True)
                o = lax.dot_general(p.astype(bf16), vb[h], NN, preferred_element_type=f32) / l
                os_[:, pl.ds(off, DH)] = o
            return c

        lax.fori_loop(done(t), done(t + 1), head, 0)
        return carry + 1

    tcount = lax.fori_loop(0, 37, body, 0)
    live = tcount > 0

    issue_slot(LAG)
    if gu_tail:
        pl.when(live)(gate_up)
        issue_slot(LAG + 1)
    pl.when(live)(down)
    issue_slot(LAG + 1 + (1 if gu_tail else 0))
    acc = jnp.zeros((1, D), f32)
    for i, nh in enumerate(CHUNKS):
        h0 = starts[i]
        with scope("wait_wo"):
            wait(wo_wait_view(h0, nh), sem.at[S_WO[i]])
        if 'h' in COMPUTE:
            def step(a):
                return a + lax.dot_general(os_[:, h0 * DH:(h0 + nh) * DH].astype(bf16),
                                           wo_rows(h0, nh), NN, preferred_element_type=f32)
            acc = lax.cond(live, step, lambda a: a, acc)
    if 'h' not in COMPUTE:
        acc = acc + qs[:, 0:512]
    ob[...] = (x + acc * gs[...]).astype(bf16).reshape(1, 1, D)
    with scope("out"):
        c = pltpu.make_async_copy(ob, out_hbm, sem.at[0])
        c.start()
        c.wait()


def make(G=4, GR=64, DG=2, LAGX=1, CHUNKS=(16, 8, 4, 2, 2), SLOTS=(0, 2, 4, 5, 5), GU_SLOT=None, WD_SLOT=0,
         COMPUTE='h', NOCHECK=False, SCOPES=False, WQ='c', PRE=1, VREV=0, WOPAT='seg'):
    assert sum(CHUNKS) == H and len(CHUNKS) == len(SLOTS)
    nsem = max(4, 2 + len(CHUNKS))
    @jax.jit
    def kernel(A_x, A_k_cache, A_v_cache, A_wq, A_wo, B_x, B_w_r, B_w_gate, B_w_up, B_w_down):
        SK = A_k_cache.shape[2]
        W = min(4096, max(256, SK // 4))
        hbm = pl.BlockSpec(memory_space=pltpu.HBM)
        return pl.pallas_call(
            functools.partial(_kernel, SK=SK, W=W, G=G, GR=GR, DG=DG, LAGX=LAGX, CHUNKS=CHUNKS, SLOTS=SLOTS,
                              GU_SLOT=GU_SLOT, WD_SLOT=WD_SLOT, COMPUTE=COMPUTE, SCOPES=SCOPES, WQ=WQ, PRE=PRE, VREV=VREV, WOPAT=WOPAT),
            grid=(),
            in_specs=[hbm] * 9,
            out_specs=hbm,
            out_shape=jax.ShapeDtypeStruct((1, 1, D), bf16),
            scratch_shapes=[
                pltpu.VMEM((H, W, DH), bf16), pltpu.VMEM((H, W, DH), bf16),
                pltpu.VMEM((8, 64, H * DH), bf16), pltpu.VMEM((8, 512, D), bf16),
                pltpu.VMEM((2, HF, D), bf16), pltpu.VMEM((2, HF, D), bf16), pltpu.VMEM((2, HF, D), bf16),
                pltpu.VMEM((1, 1, D), bf16), pltpu.VMEM((D,), bf16),
                pltpu.VMEM((1, H * DH), f32), pltpu.VMEM((1, H * DH), f32), pltpu.VMEM((1, F), f32), pltpu.VMEM((1, D), f32),
                pltpu.VMEM((1, 1, D), bf16),
                pltpu.SemaphoreType.DMA((nsem,)),
            ],
            compiler_params=pltpu.CompilerParams(vmem_limit_bytes=100 * 1024 * 1024, disable_bounds_checks=NOCHECK),
        )(A_x, A_k_cache, A_v_cache, A_wq.reshape(8, 64, H * DH), A_wo.reshape(8, 512, D), B_w_r,
          B_w_gate.T.reshape(2, HF, D), B_w_up.T.reshape(2, HF, D), B_w_down.reshape(2, HF, D))
    return kernel

pallas_recurrent_scan__sliding_block_cached__moe_arch_mod__decode_kernel = make()
```

```python
import functools

import jax
import jax.numpy as jnp
from jax import lax
import jax.experimental.pallas as pl
import jax.experimental.pallas.tpu as pltpu

D = 512
H = 32
DH = 128
F = 1376
HF = F // 2
NT = (((1,), (1,)), ((), ()))
NN = (((1,), (0,)), ((), ()))
f32 = jnp.float32
bf16 = jnp.bfloat16

ROWS = 64
N8 = 24
NITER = H + 5
WO_CHUNKS = ((0, 16, 0, 2), (16, 8, 2, 0), (24, 4, 4, 3), (28, 4, 5, 4))
S_WQ, S_GU, S_WD = 2, 3, 1
NSEM = 5


def _kernel(x_hbm, k_hbm, v_hbm, wq_hbm, wo_hbm, wr_hbm, wg_hbm, wu_hbm, wd_hbm,
            out_hbm,
            kb, vb, wqb, wob, wgb, wub, wdb, xb, wrb, qs, os_, hs, gs, ob, sem,
            *, SK, W, chunks):
    base = SK - W

    def start(src, dst, s, queue):
        pltpu.make_async_copy(src, dst, s).start(priority=queue)

    def wait(dst, s):
        pltpu.make_async_copy(dst, dst, s).wait()

    def issue_wq(s):
        start(x_hbm, xb, s, 0)
        start(wr_hbm, wrb, s, 1)

        def step(j, c):
            r = pl.multiple_of((j // 16) * 16, 16)
            c0 = pl.multiple_of(((j % 16) // 4) * 1024, 1024)
            for p in range(2):
                sg = 4 * p + j % 4
                start(wq_hbm.at[sg, pl.ds(r, 16), pl.ds(c0, 1024)],
                      wqb.at[sg, pl.ds(r, 16), pl.ds(c0, 1024)], s, p)
            return c
        lax.fori_loop(0, 64, step, 0)

    def issue_gate_up(s):
        def step(j, c):
            r = pl.multiple_of(j * 16, 16)
            start(wg_hbm.at[:, pl.ds(r, 16), :], wgb.at[:, pl.ds(r, 16), :], s, 0)
            start(wu_hbm.at[:, pl.ds(r, 16), :], wub.at[:, pl.ds(r, 16), :], s, 1)
            return c
        lax.fori_loop(0, HF // 16, step, 0)

    def issue_down(s):
        def step(j, c):
            for p in range(2):
                r = pl.multiple_of((2 * j + p) * 16, 16)
                start(wd_hbm.at[:, pl.ds(r, 16), :], wdb.at[:, pl.ds(r, 16), :], s, p)
            return c
        lax.fori_loop(0, HF // 32, step, 0)
        r = HF // 32 * 32
        start(wd_hbm.at[:, pl.ds(r, 16), :], wdb.at[:, pl.ds(r, 16), :], s, 0)

    def issue_kv(h0, r0, ng, s):
        def step(j, c):
            o = pl.multiple_of(r0 + j * ROWS, ROWS)
            for d in range(ng // 2):
                hh = h0 + 2 * d
                start(k_hbm.at[0, pl.ds(hh, 2), pl.ds(base + o, ROWS), :],
                      kb.at[pl.ds(hh, 2), pl.ds(o, ROWS), :], s, 0)
                start(v_hbm.at[0, pl.ds(hh, 2), pl.ds(base + o, ROWS), :],
                      vb.at[pl.ds(hh, 2), pl.ds(o, ROWS), :], s, 1)
            return c
        lax.fori_loop(0, W // ng // ROWS, step, 0)

    def kv_sem(i):
        return sem.at[jnp.where(i < N8, i // 8, N8 // 8 + (i - N8) // 4) % 2]

    def issue_wo(h0, nh, s):
        sg0 = h0 // 4
        if nh == 16:
            def step(j, c):
                r = pl.multiple_of(j * 16, 16)
                for p in range(2):
                    start(wo_hbm.at[pl.ds(sg0 + 2 * p, 2), pl.ds(r, 16), :],
                          wob.at[pl.ds(sg0 + 2 * p, 2), pl.ds(r, 16), :], s, p)
                return c
            lax.fori_loop(0, 32, step, 0)
        elif nh == 8:
            for j in range(32):
                start(wo_hbm.at[pl.ds(sg0, 2), pl.ds(j * 16, 16), :],
                      wob.at[pl.ds(sg0, 2), pl.ds(j * 16, 16), :], s, j % 2)
        else:
            for j in range(nh * 4):
                row = h0 * DH + j * 32
                start(wo_hbm.at[row // 512, pl.ds(row % 512, 32), :],
                      wob.at[row // 512, pl.ds(row % 512, 32), :], s, j % 2)

    def wo_view(h0, nh):
        sg0, r0 = h0 * DH // 512, h0 * DH % 512
        if nh % 4 == 0:
            return wob.at[pl.ds(sg0, nh // 4)]
        return wob.at[sg0, pl.ds(r0, nh * DH), :]

    def issue_slot(tt):
        if tt == 0:
            issue_down(sem.at[S_WD])
        for h0, nh, slot, s in chunks:
            if slot == tt:
                issue_wo(h0, nh, sem.at[s])

    issue_wq(sem.at[S_WQ])
    issue_gate_up(sem.at[S_GU])
    issue_kv(0, 0, 8, sem.at[0])

    wait(wqb, sem.at[S_WQ])
    wait(xb, sem.at[S_WQ])
    wait(wrb, sem.at[S_WQ])
    x = xb[0].astype(f32)
    xc = x - jnp.mean(x, axis=-1, keepdims=True)
    var = jnp.mean(xc * xc, axis=-1, keepdims=True)
    xn = (xc / jnp.sqrt(var + 1e-5)).astype(bf16)
    qs[...] = lax.dot_general(xn, wqb[...].reshape(D, H * DH), NN, preferred_element_type=f32)

    def gate_up():
        wait(wgb, sem.at[S_GU])
        wait(wub, sem.at[S_GU])
        gate = lax.dot_general(xn, wgb[...].reshape(F, D), NT, preferred_element_type=f32)
        up = lax.dot_general(xn, wub[...].reshape(F, D), NT, preferred_element_type=f32)
        hs[...] = gate * jax.nn.sigmoid(gate) * up

    def down():
        wait(wdb, sem.at[S_WD])
        xf = xn.astype(f32)
        y = lax.dot_general(hs[...].astype(bf16), wdb[...].reshape(F, D), NN,
                            preferred_element_type=f32)
        r = jnp.sum(xf * wrb[...].astype(f32).reshape(1, D), axis=-1, keepdims=True)
        z = xf + (xf * 0.0 + y * jax.nn.sigmoid(r))
        gs[...] = z * jax.nn.sigmoid(z)

    def head(h, c):
        @pl.when(jnp.logical_and(h < N8, h % 8 == 0))
        def _():
            wait(kb.at[pl.ds(h, 8)], kv_sem(h))
            wait(vb.at[pl.ds(h, 8)], kv_sem(h))

        @pl.when(jnp.logical_and(h >= N8, h % 4 == 0))
        def _():
            wait(kb.at[pl.ds(h, 4)], kv_sem(h))
            wait(vb.at[pl.ds(h, 4)], kv_sem(h))

        off = pl.multiple_of(h * DH, DH)
        q = qs[:, pl.ds(off, DH)].astype(bf16)
        s = lax.dot_general(q, kb[h], NT, preferred_element_type=f32) * (DH ** -0.5)
        p = jnp.exp(s - jnp.max(s, axis=-1, keepdims=True))
        l = jnp.sum(p, axis=-1, keepdims=True)
        o = lax.dot_general(p.astype(bf16), vb[h], NN, preferred_element_type=f32)
        os_[:, pl.ds(off, DH)] = o / l
        return c

    def heads_done(u):
        return jnp.where(u <= 25, jnp.maximum(u - 9, 0),
                         jnp.where(u <= 29, 16 + 2 * (u - 25), 24 + (u - 29)))

    def body(t, c):
        @pl.when(jnp.logical_and(t >= 1, t < N8))
        def _():
            issue_kv((t // 8) * 8, (t % 8) * (W // 8), 8, kv_sem(t))

        @pl.when(jnp.logical_and(t >= N8, t < H))
        def _():
            issue_kv((t // 4) * 4, (t % 4) * (W // 4), 4, kv_sem(t))

        for tt in sorted({0} | {ch[2] for ch in chunks}):
            if tt < NITER - H:
                @pl.when(t == H + tt)
                def _():
                    issue_slot(tt)

        pl.when(t == 1)(gate_up)
        lax.fori_loop(heads_done(t), heads_done(t + 1), head, 0)
        return c + 1

    live = lax.fori_loop(0, NITER, body, 0) > 0

    issue_slot(NITER - H)
    pl.when(live)(down)
    issue_slot(NITER - H + 1)
    g = gs[...]
    acc = jnp.zeros((1, D), f32)
    for h0, nh, _, s in chunks:
        o = os_[:, h0 * DH:(h0 + nh) * DH].astype(bf16)
        wait(wo_view(h0, nh), sem.at[s])

        def step(a, o=o, h0=h0, nh=nh):
            w = wo_view(h0, nh)[...].reshape(nh * DH, D)
            return a + lax.dot_general(o, w, NN, preferred_element_type=f32)
        acc = lax.cond(live, step, lambda a: a, acc) if nh >= 8 else step(acc)

    ob[...] = (x + acc * g).astype(bf16).reshape(1, 1, D)
    out = pltpu.make_async_copy(ob, out_hbm, sem.at[0])
    out.start()
    out.wait()


def make(chunks=WO_CHUNKS, nsem=NSEM):
    @jax.jit
    def kernel(A_x, A_k_cache, A_v_cache, A_wq, A_wo, B_x, B_w_r, B_w_gate, B_w_up, B_w_down):
        del B_x
        SK = A_k_cache.shape[2]
        W = min(4096, max(256, SK // 4))
        assert A_k_cache.shape == (1, H, SK, DH) and W == 4096
        hbm = pl.BlockSpec(memory_space=pltpu.HBM)
        return pl.pallas_call(
            functools.partial(_kernel, SK=SK, W=W, chunks=chunks),
            grid=(),
            in_specs=[hbm] * 9,
            out_specs=hbm,
            out_shape=jax.ShapeDtypeStruct((1, 1, D), bf16),
            scratch_shapes=[
                pltpu.VMEM((H, W, DH), bf16),
                pltpu.VMEM((H, W, DH), bf16),
                pltpu.VMEM((8, D // 8, H * DH), bf16),
                pltpu.VMEM((8, H * DH // 8, D), bf16),
                pltpu.VMEM((2, HF, D), bf16),
                pltpu.VMEM((2, HF, D), bf16),
                pltpu.VMEM((2, HF, D), bf16),
                pltpu.VMEM((1, 1, D), bf16),
                pltpu.VMEM((D,), bf16),
                pltpu.VMEM((1, H * DH), f32),
                pltpu.VMEM((1, H * DH), f32),
                pltpu.VMEM((1, F), f32),
                pltpu.VMEM((1, D), f32),
                pltpu.VMEM((1, 1, D), bf16),
                pltpu.SemaphoreType.DMA((nsem,)),
            ],
            compiler_params=pltpu.CompilerParams(vmem_limit_bytes=100 * 1024 * 1024),
        )(A_x, A_k_cache, A_v_cache,
          A_wq.reshape(8, D // 8, H * DH), A_wo.reshape(8, H * DH // 8, D), B_w_r,
          B_w_gate.T.reshape(2, HF, D), B_w_up.T.reshape(2, HF, D), B_w_down.reshape(2, HF, D))
    return kernel


pallas_recurrent_scan__sliding_block_cached__moe_arch_mod__decode_kernel = make()
```

```python
import functools

import jax
import jax.numpy as jnp
from jax import lax
import jax.experimental.pallas as pl
import jax.experimental.pallas.tpu as pltpu

D = 512
H = 32
DH = 128
F = 1376
HF = F // 2
NT = (((1,), (1,)), ((), ()))
NN = (((1,), (0,)), ((), ()))
f32 = jnp.float32
bf16 = jnp.bfloat16

ROWS = 64
N8 = 24
NITER = H + 5
WO_CHUNKS = ((0, 16, 0, 2), (16, 8, 2, 0), (24, 4, 4, 3), (28, 4, 5, 4))
S_WQ, S_GU, S_WD = 2, 3, 1
NSEM = 5


def _kernel(x_hbm, k_hbm, v_hbm, wq_hbm, wo_hbm, wr_hbm, wg_hbm, wu_hbm, wd_hbm,
            out_hbm,
            kb, vb, wqb, wob, wgb, wub, wdb, xb, wrb, qs, os_, hs, gs, ob, sem,
            *, SK, W):
    base = SK - W

    def start(src, dst, s, queue):
        pltpu.make_async_copy(src, dst, s).start(priority=queue)

    def wait(dst, s):
        pltpu.make_async_copy(dst, dst, s).wait()

    def issue_wq(s):
        start(x_hbm, xb, s, 0)
        start(wr_hbm, wrb, s, 1)

        def step(j, c):
            r = pl.multiple_of((j // 16) * 16, 16)
            c0 = pl.multiple_of(((j % 16) // 4) * 1024, 1024)
            for p in range(2):
                sg = 4 * p + j % 4
                start(wq_hbm.at[sg, pl.ds(r, 16), pl.ds(c0, 1024)],
                      wqb.at[sg, pl.ds(r, 16), pl.ds(c0, 1024)], s, p)
            return c
        lax.fori_loop(0, 64, step, 0)

    def issue_gate_up(s):
        def step(j, c):
            r = pl.multiple_of(j * 16, 16)
            start(wg_hbm.at[:, pl.ds(r, 16), :], wgb.at[:, pl.ds(r, 16), :], s, 0)
            start(wu_hbm.at[:, pl.ds(r, 16), :], wub.at[:, pl.ds(r, 16), :], s, 1)
            return c
        lax.fori_loop(0, HF // 16, step, 0)

    def issue_down(s):
        def step(j, c):
            for p in range(2):
                r = pl.multiple_of((2 * j + p) * 16, 16)
                start(wd_hbm.at[:, pl.ds(r, 16), :], wdb.at[:, pl.ds(r, 16), :], s, p)
            return c
        lax.fori_loop(0, HF // 32, step, 0)
        r = HF // 32 * 32
        start(wd_hbm.at[:, pl.ds(r, 16), :], wdb.at[:, pl.ds(r, 16), :], s, 0)

    def issue_kv(h0, r0, ng, s):
        def step(j, c):
            o = pl.multiple_of(r0 + j * ROWS, ROWS)
            for d in range(ng // 2):
                hh = h0 + 2 * d
                start(k_hbm.at[0, pl.ds(hh, 2), pl.ds(base + o, ROWS), :],
                      kb.at[pl.ds(hh, 2), pl.ds(o, ROWS), :], s, 0)
                start(v_hbm.at[0, pl.ds(hh, 2), pl.ds(base + o, ROWS), :],
                      vb.at[pl.ds(hh, 2), pl.ds(o, ROWS), :], s, 1)
            return c
        lax.fori_loop(0, W // ng // ROWS, step, 0)

    def kv_sem(i):
        return sem.at[jnp.where(i < N8, i // 8, N8 // 8 + (i - N8) // 4) % 2]

    def issue_wo(h0, nh, s):
        sg0 = h0 // 4
        if nh == 16:
            def step(j, c):
                r = pl.multiple_of(j * 16, 16)
                for p in range(2):
                    start(wo_hbm.at[pl.ds(sg0 + 2 * p, 2), pl.ds(r, 16), :],
                          wob.at[pl.ds(sg0 + 2 * p, 2), pl.ds(r, 16), :], s, p)
                return c
            lax.fori_loop(0, 32, step, 0)
        elif nh == 8:
            for j in range(32):
                start(wo_hbm.at[pl.ds(sg0, 2), pl.ds(j * 16, 16), :],
                      wob.at[pl.ds(sg0, 2), pl.ds(j * 16, 16), :], s, j % 2)
        else:
            for j in range(nh * 4):
                row = h0 * DH + j * 32
                start(wo_hbm.at[row // 512, pl.ds(row % 512, 32), :],
                      wob.at[row // 512, pl.ds(row % 512, 32), :], s, j % 2)

    def wo_view(h0, nh):
        sg0, r0 = h0 * DH // 512, h0 * DH % 512
        if nh % 4 == 0:
            return wob.at[pl.ds(sg0, nh // 4)]
        return wob.at[sg0, pl.ds(r0, nh * DH), :]

    def issue_slot(tt):
        if tt == 0:
            issue_down(sem.at[S_WD])
        for h0, nh, slot, s in WO_CHUNKS:
            if slot == tt:
                issue_wo(h0, nh, sem.at[s])

    issue_wq(sem.at[S_WQ])
    issue_gate_up(sem.at[S_GU])
    issue_kv(0, 0, 8, sem.at[0])

    wait(wqb, sem.at[S_WQ])
    wait(xb, sem.at[S_WQ])
    wait(wrb, sem.at[S_WQ])
    x = xb[0].astype(f32)
    xc = x - jnp.mean(x, axis=-1, keepdims=True)
    var = jnp.mean(xc * xc, axis=-1, keepdims=True)
    xn = (xc / jnp.sqrt(var + 1e-5)).astype(bf16)
    qs[...] = lax.dot_general(xn, wqb[...].reshape(D, H * DH), NN, preferred_element_type=f32)

    def gate_up():
        wait(wgb, sem.at[S_GU])
        wait(wub, sem.at[S_GU])
        gate = lax.dot_general(xn, wgb[...].reshape(F, D), NT, preferred_element_type=f32)
        up = lax.dot_general(xn, wub[...].reshape(F, D), NT, preferred_element_type=f32)
        hs[...] = gate * jax.nn.sigmoid(gate) * up

    def down():
        wait(wdb, sem.at[S_WD])
        xf = xn.astype(f32)
        y = lax.dot_general(hs[...].astype(bf16), wdb[...].reshape(F, D), NN,
                            preferred_element_type=f32)
        r = jnp.sum(xf * wrb[...].astype(f32).reshape(1, D), axis=-1, keepdims=True)
        z = xf + (xf * 0.0 + y * jax.nn.sigmoid(r))
        gs[...] = z * jax.nn.sigmoid(z)

    def head(h, c):
        @pl.when(jnp.logical_and(h < N8, h % 8 == 0))
        def _():
            wait(kb.at[pl.ds(h, 8)], kv_sem(h))
            wait(vb.at[pl.ds(h, 8)], kv_sem(h))

        @pl.when(jnp.logical_and(h >= N8, h % 4 == 0))
        def _():
            wait(kb.at[pl.ds(h, 4)], kv_sem(h))
            wait(vb.at[pl.ds(h, 4)], kv_sem(h))

        off = pl.multiple_of(h * DH, DH)
        q = qs[:, pl.ds(off, DH)].astype(bf16)
        s = lax.dot_general(q, kb[h], NT, preferred_element_type=f32) * (DH ** -0.5)
        p = jnp.exp(s - jnp.max(s, axis=-1, keepdims=True))
        l = jnp.sum(p, axis=-1, keepdims=True)
        o = lax.dot_general(p.astype(bf16), vb[h], NN, preferred_element_type=f32)
        os_[:, pl.ds(off, DH)] = o / l
        return c

    def heads_done(u):
        return jnp.where(u <= 25, jnp.maximum(u - 9, 0),
                         jnp.where(u <= 29, 16 + 2 * (u - 25), 24 + (u - 29)))

    def body(t, c):
        @pl.when(jnp.logical_and(t >= 1, t < N8))
        def _():
            issue_kv((t // 8) * 8, (t % 8) * (W // 8), 8, kv_sem(t))

        @pl.when(jnp.logical_and(t >= N8, t < H))
        def _():
            issue_kv((t // 4) * 4, (t % 4) * (W // 4), 4, kv_sem(t))

        for tt in sorted({0} | {ch[2] for ch in WO_CHUNKS}):
            if tt < NITER - H:
                @pl.when(t == H + tt)
                def _():
                    issue_slot(tt)

        pl.when(t == 1)(gate_up)
        lax.fori_loop(heads_done(t), heads_done(t + 1), head, 0)
        return c + 1

    live = lax.fori_loop(0, NITER, body, 0) > 0

    issue_slot(NITER - H)
    pl.when(live)(down)
    issue_slot(NITER - H + 1)
    g = gs[...]
    acc = jnp.zeros((1, D), f32)
    for h0, nh, _, s in WO_CHUNKS:
        o = os_[:, h0 * DH:(h0 + nh) * DH].astype(bf16)
        wait(wo_view(h0, nh), sem.at[s])

        def step(a, o=o, h0=h0, nh=nh):
            w = wo_view(h0, nh)[...].reshape(nh * DH, D)
            return a + lax.dot_general(o, w, NN, preferred_element_type=f32)
        acc = lax.cond(live, step, lambda a: a, acc) if nh >= 8 else step(acc)

    ob[...] = (x + acc * g).astype(bf16).reshape(1, 1, D)
    out = pltpu.make_async_copy(ob, out_hbm, sem.at[0])
    out.start()
    out.wait()


@jax.jit
def pallas_recurrent_scan__sliding_block_cached__moe_arch_mod__decode_kernel(
    A_x: jax.Array,
    A_k_cache: jax.Array,
    A_v_cache: jax.Array,
    A_wq: jax.Array,
    A_wo: jax.Array,
    B_x: jax.Array,
    B_w_r: jax.Array,
    B_w_gate: jax.Array,
    B_w_up: jax.Array,
    B_w_down: jax.Array,
):
    del B_x
    SK = A_k_cache.shape[2]
    W = min(4096, max(256, SK // 4))
    assert A_k_cache.shape == (1, H, SK, DH) and W == 4096
    hbm = pl.BlockSpec(memory_space=pltpu.HBM)
    return pl.pallas_call(
        functools.partial(_kernel, SK=SK, W=W),
        grid=(),
        in_specs=[hbm] * 9,
        out_specs=hbm,
        out_shape=jax.ShapeDtypeStruct((1, 1, D), bf16),
        scratch_shapes=[
            pltpu.VMEM((H, W, DH), bf16),
            pltpu.VMEM((H, W, DH), bf16),
            pltpu.VMEM((8, D // 8, H * DH), bf16),
            pltpu.VMEM((8, H * DH // 8, D), bf16),
            pltpu.VMEM((2, HF, D), bf16),
            pltpu.VMEM((2, HF, D), bf16),
            pltpu.VMEM((2, HF, D), bf16),
            pltpu.VMEM((1, 1, D), bf16),
            pltpu.VMEM((D,), bf16),
            pltpu.VMEM((1, H * DH), f32),
            pltpu.VMEM((1, H * DH), f32),
            pltpu.VMEM((1, F), f32),
            pltpu.VMEM((1, D), f32),
            pltpu.VMEM((1, 1, D), bf16),
            pltpu.SemaphoreType.DMA((NSEM,)),
        ],
        compiler_params=pltpu.CompilerParams(vmem_limit_bytes=100 * 1024 * 1024),
    )(A_x, A_k_cache, A_v_cache,
      A_wq.reshape(8, D // 8, H * DH), A_wo.reshape(8, H * DH // 8, D), B_w_r,
      B_w_gate.T.reshape(2, HF, D), B_w_up.T.reshape(2, HF, D), B_w_down.reshape(2, HF, D))
```
